```python
import os as _os
_os.environ.setdefault("JAX_PLATFORMS", "cpu")
import jax
import jax.numpy as jnp

def _softmax(x, axis=-1):
    return jax.nn.softmax(x, axis=axis)
def _gelu(x):
    return jax.nn.gelu(x, approximate=True)
def _silu(x):
    return jax.nn.silu(x)
def _sigmoid(x):
    return jax.nn.sigmoid(x)
def _layernorm(x, axis=-1, eps=1e-5):
    m = jnp.mean(x, axis=axis, keepdims=True)
    v = jnp.var(x, axis=axis, keepdims=True)
    return (x - m) / jnp.sqrt(v + eps)
def _scatter_add(tgt, idx, src, axis=0):
    return tgt.at[idx].add(src)
def _segment_sum(src, seg, n):
    return jax.ops.segment_sum(src, seg, n)
class _Rng:
    def __init__(self, key):
        self._k = key
    def _next(self):
        self._k, sub = jax.random.split(self._k)
        return sub
    def normal(self, shape):
        return jax.random.normal(self._next(), shape, dtype=jnp.bfloat16)
    def randint(self, lo, hi, shape):
        return jax.random.randint(self._next(), shape, lo, hi, dtype=jnp.int32)
    def uniform(self, shape, lo=0.0, hi=1.0):
        return jax.random.uniform(self._next(), shape, jnp.bfloat16, lo, hi)
    def permutation(self, n):
        return jax.random.permutation(self._next(), n)


kernel_name = 'standalone__groupnorm__sampling'

def setup_inputs():
    _rng = _Rng(jax.random.key(int.from_bytes(__import__("os").urandom(4), "little")))
    _w = (lambda a: (lambda t: t.astype(jnp.bfloat16) if jnp.issubdtype(t.dtype, jnp.floating) else t)(jnp.asarray(a)))
    B = 32
    G = 32
    cpg = max(1, 576 // G)
    C = G * cpg
    H, W = 32, 16
    return {
        "x": _w((lambda *s: _rng.normal(s) * 0.05)(B, C, H, W)),
        "g": _w((lambda *s: _rng.normal(s) * 0.05)(C) + 1.0),
        "b": _w((lambda *s: _rng.normal(s) * 0.05)(C)),
    }

def reference(x, g, b):
    G = 32
    B, C, H, W = x.shape[0], x.shape[1], x.shape[2], x.shape[3]
    xr = x.reshape(B, G, C // G, H, W)
    mu = xr.mean(axis=(2, 3, 4), keepdims=True)
    var = ((xr - mu) ** 2).mean(axis=(2, 3, 4), keepdims=True)
    xn = (xr - mu) / jnp.sqrt(var + 1e-5)
    xn = xn.reshape(B, C, H, W)
    return xn * g[None, :, None, None] + b[None, :, None, None]
```

```python
import functools

import jax
import jax.numpy as jnp
from jax import lax
import jax.experimental.pallas as pl
import jax.experimental.pallas.tpu as pltpu

_GROUPS = 32
_EPS = 1e-5
_LANES = 128
_STREAMS = 8
_TAIL_ROWS = 20
_UNROLL = 4


def _group_total(v, pos, cpg):
    width = v.shape[-1]

    def shifted(a, s):
        return jnp.where(
            pos >= s,
            pltpu.roll(a, s, 1),
            pltpu.roll(a, (width + s - cpg) % width, 1),
        )

    step, factor = cpg, 2
    while step > 1:
        while step % factor:
            factor += 1
        step //= factor
        total = v
        for m in range(1, factor):
            total = total + shifted(v, m * step)
        v = total
    return v


def _kernel(x_hbm, g_hbm, b_hbm, o_hbm, buf, g_vmem, b_vmem, stat, scale,
            rsem, psem, wsem, *, cpg, tail):
    streams, parts, height, width, chans = buf.shape
    padded = stat.shape[1]
    inv_count = 1.0 / (cpg * height * width)
    last = parts - 1

    def read(idx, sem):
        return pltpu.make_async_copy(x_hbm.at[idx], buf.at[idx], rsem.at[sem])

    reads = [read((slice(None), q), q) for q in range(last)]
    last_reads = [
        read((pl.ds(0, streams - 1), last), last),
        read((streams - 1, last, pl.ds(0, height - tail)), last),
    ]
    tail_read = read((streams - 1, last, pl.ds(height - tail, tail)), parts)
    params = [
        pltpu.make_async_copy(g_hbm, g_vmem, psem.at[0]),
        pltpu.make_async_copy(b_hbm, b_vmem, psem.at[1]),
    ]
    reads[0].start()
    for copy in params + reads[1:] + last_reads + [tail_read]:
        copy.start()

    lane = lax.broadcasted_iota(jnp.int32, (streams, padded), 1)
    pos = lax.rem(lane, cpg)
    stat[...] = jnp.zeros(stat.shape, jnp.float32)
    for copy in params:
        copy.wait()
    gamma = g_vmem[...].astype(jnp.float32).reshape(1, chans)
    beta = b_vmem[...].astype(jnp.float32).reshape(1, chans)

    def column_sums(q, term):
        @pl.loop(0, streams)
        def _(k):
            fn = term(k)

            def body(h, acc):
                return acc + fn(buf[k, q, h].astype(jnp.float32))

            acc = lax.fori_loop(
                0, height, body, jnp.zeros((width, chans), jnp.float32),
                unroll=_UNROLL)
            stat[pl.ds(k, 1), pl.ds(0, chans)] = jnp.sum(
                acc, axis=0, keepdims=True)

    def normalise(q):
        column_sums(q, lambda k: lambda x: x)
        mean = _group_total(stat[...], pos, cpg) * inv_count
        scale[0] = mean

        def row(i, k):
            return jnp.broadcast_to(
                scale[i, pl.ds(k, 1), pl.ds(0, chans)], (width, chans))

        def squared_deviation(k):
            mu = row(0, k)
            return lambda x: (x - mu) * (x - mu)

        column_sums(q, squared_deviation)
        var = _group_total(stat[...], pos, cpg) * inv_count
        scale[1, :, pl.ds(0, chans)] = lax.rsqrt(var + _EPS)[:, :chans] * gamma

        @pl.loop(0, streams)
        def _(k):
            mu, a = row(0, k), row(1, k)
            c = jnp.broadcast_to(beta, (width, chans))

            @pl.loop(0, height, unroll=_UNROLL)
            def _(h):
                x = buf[k, q, h].astype(jnp.float32)
                buf[k, q, h] = ((x - mu) * a + c).astype(buf.dtype)

    def write(first_part, num_parts):
        @pl.loop(first_part * height, (first_part + num_parts) * height)
        def _(i):
            idx = (slice(None), i // height, i % height)
            pltpu.make_async_copy(buf.at[idx], o_hbm.at[idx], wsem).start()

    @pl.loop(0, parts)
    def _(q):
        @pl.when(q < last)
        def _():
            read((slice(None), q), q).wait()

        @pl.when(q == last)
        def _():
            for copy in last_reads:
                copy.wait()
            write(0, 1)
            tail_read.wait()

        normalise(q)

    write(1, last)
    pltpu.make_async_copy(buf, o_hbm, wsem).wait()


@jax.jit
def pallas_standalone__groupnorm__sampling_kernel(
    x: jax.Array,
    g: jax.Array,
    b: jax.Array,
):
    batch, chans, height, width = x.shape
    parts = batch // _STREAMS
    assert parts * _STREAMS == batch and parts > 1 and chans % _GROUPS == 0
    padded = pl.cdiv(chans, _LANES) * _LANES
    shape = (_STREAMS, parts, height, width, chans)
    in_hbm = pl.BlockSpec(memory_space=pl.ANY)

    out = pl.pallas_call(
        functools.partial(
            _kernel, cpg=chans // _GROUPS, tail=min(_TAIL_ROWS, height - 1)),
        out_shape=jax.ShapeDtypeStruct(shape, x.dtype),
        in_specs=[in_hbm, in_hbm, in_hbm],
        out_specs=in_hbm,
        scratch_shapes=[
            pltpu.VMEM(shape, x.dtype),
            pltpu.VMEM((chans,), g.dtype),
            pltpu.VMEM((chans,), b.dtype),
            pltpu.VMEM((_STREAMS, padded), jnp.float32),
            pltpu.VMEM((2, _STREAMS, padded), jnp.float32),
            pltpu.SemaphoreType.DMA((parts + 1,)),
            pltpu.SemaphoreType.DMA((2,)),
            pltpu.SemaphoreType.DMA(()),
        ],
        compiler_params=pltpu.CompilerParams(
            vmem_limit_bytes=64 * 1024 * 1024,
            disable_bounds_checks=True,
        ),
    )(jnp.transpose(x, (0, 2, 3, 1)).reshape(shape), g, b)
    return jnp.transpose(out.reshape(batch, height, width, chans), (0, 3, 1, 2))
```

```python
import functools

import jax
import jax.numpy as jnp
from jax import lax
import jax.experimental.pallas as pl
import jax.experimental.pallas.tpu as pltpu

_GROUPS = 32
_EPS = 1e-5
_LANES = 128
_STREAMS = 8
_TAIL_ROWS = 20
_UNROLL = 4


def _group_total(v, pos, cpg):
    width = v.shape[-1]

    def shifted(a, s):
        return jnp.where(
            pos >= s,
            pltpu.roll(a, s, 1),
            pltpu.roll(a, (width + s - cpg) % width, 1),
        )

    step, factor = cpg, 2
    while step > 1:
        while step % factor:
            factor += 1
        step //= factor
        total = v
        for m in range(1, factor):
            total = total + shifted(v, m * step)
        v = total
    return v


def _kernel(x_hbm, g_hbm, b_hbm, o_hbm, buf, g_vmem, b_vmem, stat, coef,
            rsem, psem, wsem, *, cpg, tail):
    streams, parts, height, width, chans = buf.shape
    padded = stat.shape[1]
    inv_count = 1.0 / (cpg * height * width)
    last = parts - 1
    early = parts // 2

    def read(idx, sem):
        return pltpu.make_async_copy(x_hbm.at[idx], buf.at[idx], rsem.at[sem])

    params = [
        pltpu.make_async_copy(g_hbm, g_vmem, psem.at[0]),
        pltpu.make_async_copy(b_hbm, b_vmem, psem.at[1]),
    ]
    last_reads = [
        read((pl.ds(0, streams - 1), last), last),
        read((streams - 1, last, pl.ds(0, height - tail)), last),
    ]
    tail_read = read((streams - 1, last, pl.ds(height - tail, tail)), parts)

    for copy in params:
        copy.start()

    @pl.loop(0, last)
    def _(q):
        read((slice(None), q), q).start()

    for copy in last_reads + [tail_read]:
        copy.start()

    lane = lax.broadcasted_iota(jnp.int32, (streams, padded), 1)
    pos = lax.rem(lane, cpg)
    stat[...] = jnp.zeros(stat.shape, jnp.float32)
    for copy in params:
        copy.wait()
    gamma = g_vmem[...].astype(jnp.float32).reshape(1, chans)
    beta = b_vmem[...].astype(jnp.float32).reshape(1, chans)

    def group_mean(q, term):
        @pl.loop(0, streams)
        def _(k):
            fn = term(k)

            def body(h, acc):
                return acc + fn(buf[k, q, h].astype(jnp.float32))

            acc = lax.fori_loop(
                0, height, body, jnp.zeros((width, chans), jnp.float32),
                unroll=_UNROLL)
            stat[pl.ds(k, 1), pl.ds(0, chans)] = jnp.sum(
                acc, axis=0, keepdims=True)

        return _group_total(stat[...], pos, cpg) * inv_count

    def coef_row(i, k):
        return jnp.broadcast_to(
            coef[i, pl.ds(k, 1), pl.ds(0, chans)], (width, chans))

    def squared_deviation(k):
        mu = coef_row(0, k)
        return lambda x: (x - mu) * (x - mu)

    def normalise(q):
        coef[0] = group_mean(q, lambda k: lambda x: x)
        var = group_mean(q, squared_deviation)
        coef[1, :, pl.ds(0, chans)] = lax.rsqrt(var + _EPS)[:, :chans] * gamma

        @pl.loop(0, streams)
        def _(k):
            mu, scale = coef_row(0, k), coef_row(1, k)
            shift = jnp.broadcast_to(beta, (width, chans))

            @pl.loop(0, height, unroll=_UNROLL)
            def _(h):
                x = buf[k, q, h].astype(jnp.float32)
                buf[k, q, h] = ((x - mu) * scale + shift).astype(buf.dtype)

    def write(first_part, end_part):
        @pl.loop(first_part * height, end_part * height)
        def _(i):
            idx = (slice(None), lax.div(i, height), lax.rem(i, height))
            pltpu.make_async_copy(buf.at[idx], o_hbm.at[idx], wsem).start()

    @pl.loop(0, parts)
    def _(q):
        @pl.when(q < last)
        def _():
            read((slice(None), q), q).wait()

        @pl.when(q == early)
        def _():
            for copy in last_reads:
                copy.wait()
            write(0, early)
            tail_read.wait()

        normalise(q)

        @pl.when(q >= early)
        def _():
            write(q, q + 1)

    pltpu.make_async_copy(buf, o_hbm, wsem).wait()


@jax.jit
def pallas_standalone__groupnorm__sampling_kernel(
    x: jax.Array,
    g: jax.Array,
    b: jax.Array,
):
    batch, chans, height, width = x.shape
    parts = batch // _STREAMS
    assert parts * _STREAMS == batch and parts > 1 and chans % _GROUPS == 0
    padded = pl.cdiv(chans, _LANES) * _LANES
    shape = (_STREAMS, parts, height, width, chans)
    in_hbm = pl.BlockSpec(memory_space=pl.ANY)

    out = pl.pallas_call(
        functools.partial(
            _kernel, cpg=chans // _GROUPS, tail=min(_TAIL_ROWS, height - 1)),
        out_shape=jax.ShapeDtypeStruct(shape, x.dtype),
        in_specs=[in_hbm, in_hbm, in_hbm],
        out_specs=in_hbm,
        scratch_shapes=[
            pltpu.VMEM(shape, x.dtype),
            pltpu.VMEM((chans,), g.dtype),
            pltpu.VMEM((chans,), b.dtype),
            pltpu.VMEM((_STREAMS, padded), jnp.float32),
            pltpu.VMEM((2, _STREAMS, padded), jnp.float32),
            pltpu.SemaphoreType.DMA((parts + 1,)),
            pltpu.SemaphoreType.DMA((2,)),
            pltpu.SemaphoreType.DMA(()),
        ],
        compiler_params=pltpu.CompilerParams(
            vmem_limit_bytes=64 * 1024 * 1024,
            disable_bounds_checks=True,
            disable_semaphore_checks=True,
        ),
    )(jnp.transpose(x, (0, 2, 3, 1)).reshape(shape), g, b)
    return jnp.transpose(out.reshape(batch, height, width, chans), (0, 3, 1, 2))
```

```python
import functools

import jax
import jax.numpy as jnp
from jax import lax
import jax.experimental.pallas as pl
import jax.experimental.pallas.tpu as pltpu

_GROUPS = 32
_EPS = 1e-5
_LANES = 128
_BAND = 8
_QUARTERS = 4
_UNROLL = 16

_STREAMS = 5
_STREAM_TILES = 512
_READ_TILES = 16
_WRITE_BANDS = 3
_SIDE_SLOTS = 100
_SIDE_REUSED = 8

_EARLY_IMAGES = 12
_LEAD_READS = 7
_FORWARD_ROUND = 20
_LAST_READS = 2
_MARKER_CHUNK = 2
_LEAD_WRITES = 15
_STEP_WRITES = 2

_copy = pltpu.make_async_copy


def _div(n, d):
    return lax.shift_right_logical(n * pl.cdiv(1 << 16, d), 16)


def _pieces(first, count, chans):
    boxes, end = [], first + count
    while first < end:
        band, tile = divmod(first, _STREAMS)
        if tile == 0 and end - first >= _STREAMS:
            bands = (end - first) // _STREAMS
            boxes.append((band, bands, 0, chans))
            first += bands * _STREAMS
        else:
            stop = min(_STREAMS, tile + end - first)
            lo, hi = tile * _LANES, min(stop * _LANES, chans)
            boxes.append((band, 1, lo, hi - lo))
            first += stop - tile
    return boxes


def _group_total(v, cpg):
    width = v.shape[-1]
    lane = lax.broadcasted_iota(jnp.int32, v.shape, 1)
    pos = lane - cpg * _div(lane, cpg)

    def shifted(a, s):
        return jnp.where(
            pos >= s,
            pltpu.roll(a, s, 1),
            pltpu.roll(a, (width + s - cpg) % width, 1),
        )

    step, factor = cpg, 2
    while step > 1:
        while step % factor:
            factor += 1
        step //= factor
        total = v
        for m in range(1, factor):
            total = total + shifted(v, m * step)
        v = total
    return v


def _normalise(buf, stat, gamma, beta, first, count, slots, feed, *, per_quarter):
    chans = buf.shape[-1]
    cpg = chans // _GROUPS
    bands = buf.shape[1] // per_quarter
    pixels = bands * _BAND

    def image(k):
        q = _div(first + k, per_quarter)
        return buf.at[q, pl.ds((first + k - q * per_quarter) * bands, bands)]

    @pl.loop(0, count)
    def _(k):
        img = image(k)
        pivot = img[0].astype(jnp.float32)

        def body(c, sums):
            s1, s2 = sums
            for i in range(_UNROLL):
                d = img[c * _UNROLL + i].astype(jnp.float32) - pivot
                s1, s2 = s1 + d, s2 + d * d
            return s1, s2

        zero = jnp.zeros((_BAND, chans), jnp.float32)
        s1, s2 = lax.fori_loop(0, bands // _UNROLL, body, (zero, zero))
        shift = s1 * (1.0 / bands)
        mean = pivot + shift
        m2 = jnp.where(s2 == jnp.inf, s2, s2 - s1 * shift)
        chan_mean = jnp.sum(mean, axis=0, keepdims=True) * (1.0 / _BAND)
        m2 = m2 + bands * ((mean - chan_mean) * (mean - chan_mean))
        stat[0, pl.ds(k, 1), pl.ds(0, chans)] = chan_mean
        stat[1, pl.ds(k, 1), pl.ds(0, chans)] = jnp.sum(m2, axis=0, keepdims=True)
        feed(0, k)

    chan_mean = stat[0, :slots]
    mean = _group_total(chan_mean, cpg) / cpg
    m2 = stat[1, :slots] + pixels * ((chan_mean - mean) * (chan_mean - mean))
    var = _group_total(m2, cpg) / (cpg * pixels)
    stat[2, :slots] = mean
    stat[3, :slots, :chans] = lax.rsqrt(var + _EPS)[:, :chans] * gamma

    @pl.loop(0, count)
    def _(k):
        img = image(k)
        mu, scale = (
            jnp.broadcast_to(stat[i, pl.ds(k, 1), pl.ds(0, chans)], (_BAND, chans))
            for i in (2, 3)
        )
        bias = jnp.broadcast_to(beta, (_BAND, chans))

        @pl.loop(0, bands // _UNROLL)
        def _(c):
            for i in range(_UNROLL):
                x = img[c * _UNROLL + i].astype(jnp.float32)
                img[c * _UNROLL + i] = ((x - mu) * scale + bias).astype(buf.dtype)

        feed(1, k)


def _kernel(x_hbm, g_hbm, b_hbm, o_hbm, buf, side, g_vmem, b_vmem, spare, stat,
            read_sem, param_sem, side_in_sem, side_out_sem, write_sem, *, batch):
    _, quarter, _, chans = buf.shape
    per_quarter = batch // _QUARTERS
    image_bands = quarter // per_quarter
    direct = quarter - _SIDE_SLOTS - _SIDE_REUSED
    chunked = direct // _READ_TILES * _READ_TILES
    rounds = _STREAM_TILES // _READ_TILES
    assert chunked < direct and _SIDE_REUSED < _SIDE_SLOTS + _SIDE_REUSED - image_bands
    assert _EARLY_IMAGES <= rounds - _LAST_READS - _LEAD_READS <= 2 * _EARLY_IMAGES
    assert per_quarter <= _EARLY_IMAGES < 2 * per_quarter

    def read_round(half, j, phases=range(_STREAMS)):
        for phase in phases:
            stream = 2 * j + (3 * phase) % _STREAMS
            stream = stream - _STREAMS * _div(stream, _STREAMS)
            band0 = _div(_STREAM_TILES * stream + _READ_TILES * j, _STREAMS)

            def start(quarters, sem):
                for band, bands, lo, width in _pieces(phase, _READ_TILES, chans):
                    box = (pl.ds(2 * half, quarters), pl.ds(band0 + band, bands),
                           slice(None), pl.ds(lo, width))
                    _copy(x_hbm.at[box], buf.at[box], read_sem.at[sem]).start()

            if half:
                lax.cond(band0 < chunked, lambda: start(2, 1), lambda: start(1, 2))
            else:
                start(2, 0)

    filled = [
        _copy(x_hbm.at[box], buf.at[box], read_sem.at[i])
        for i, box in enumerate([
            (pl.ds(0, 2),),
            (pl.ds(2, 2), pl.ds(0, chunked)),
            (pl.ds(2, 1), pl.ds(chunked, quarter - chunked)),
            (pl.ds(3, 1), pl.ds(chunked, direct - chunked)),
        ])
    ]

    def staged(lo, hi):
        bands = (_QUARTERS - 1, pl.ds(direct + lo, hi - lo))
        return bands, side.at[pl.ds(lo % _SIDE_SLOTS, hi - lo)]

    cuts = [0, _SIDE_REUSED, _SIDE_SLOTS, _SIDE_SLOTS + _SIDE_REUSED]
    side_in = [
        _copy(x_hbm.at[bands], slots, side_in_sem.at[i])
        for i, (bands, slots) in enumerate(map(staged, cuts, cuts[1:]))
    ]
    cuts.insert(2, quarter - image_bands - direct)
    side_out = [
        _copy(slots, buf.at[bands], side_out_sem.at[i])
        for i, (bands, slots) in enumerate(map(staged, cuts, cuts[1:]))
    ]
    params = [_copy(g_hbm, g_vmem, param_sem.at[0]),
              _copy(b_hbm, b_vmem, param_sem.at[1])]
    marker = _copy(b_hbm, spare, param_sem.at[2])

    edges = [(_STREAM_TILES * i + 2) // _STREAMS for i in range(_STREAMS + 1)]
    write_rounds = (_STREAM_TILES // _STREAMS) // _WRITE_BANDS
    assert _LEAD_WRITES <= write_rounds

    def write(lo, hi):
        @pl.loop(lo, hi)
        def _(n):
            q = _div(n, write_rounds)
            window = (q, pl.ds((n - q * write_rounds) * _WRITE_BANDS,
                               edges[-2] + _WRITE_BANDS))
            src, dst = buf.at[window], o_hbm.at[window]
            for edge in edges[:-1]:
                box = pl.ds(edge, _WRITE_BANDS)
                _copy(src.at[box], dst.at[box], write_sem).start()

    side_in[0].start()

    @pl.loop(0, rounds)
    def _(j):
        read_round(0, j)

        @pl.when(j == 1)
        def _():
            for copy in [side_in[1]] + params:
                copy.start()

        @pl.when(j == _FORWARD_ROUND)
        def _():
            side_in[0].wait()
            side_out[0].start()

    filled[3].start()
    pl.loop(0, _LEAD_READS)(functools.partial(read_round, 1))

    stat[...] = jnp.zeros(stat.shape, jnp.float32)
    for copy in params:
        copy.wait()
    normalise = functools.partial(
        _normalise, buf, stat,
        g_vmem[...].astype(jnp.float32).reshape(1, chans),
        b_vmem[...].astype(jnp.float32).reshape(1, chans),
        per_quarter=per_quarter)
    side_out[0].wait()
    side_in[2].start()
    filled[0].wait()

    def feed_reads(stage, k):
        j = _LEAD_READS + stage * _EARLY_IMAGES + k
        if stage == 0:
            read_round(1, j)
        else:
            pl.when(j < rounds - _LAST_READS)(lambda: read_round(1, j))

    normalise(0, _EARLY_IMAGES, stat.shape[1], feed_reads)

    @pl.loop(rounds - _LAST_READS, rounds)
    def _(j):
        read_round(1, j, range(_MARKER_CHUNK))

        @pl.loop(0, 2)
        def _(i):
            pl.when(i + j == rounds - _LAST_READS)(marker.start)

        read_round(1, j, range(_MARKER_CHUNK, _STREAMS))

    side_in[1].wait()
    side_in[2].wait()

    @pl.loop(1, len(side_out))
    def _(i):
        for n in range(1, len(side_out)):
            pl.when(i == n)(side_out[n].start)

    marker.wait()
    write(0, _LEAD_WRITES)
    for copy in filled[1:]:
        copy.wait()

    starts = [_EARLY_IMAGES, 2 * per_quarter, 3 * per_quarter, batch - 1, batch]
    before_last = (_QUARTERS - 1) * write_rounds + (
        quarter - image_bands - edges[-2]) // _WRITE_BANDS

    def step(u, sent):
        first, count = starts[0], starts[1] - starts[0]
        for i in range(1, len(starts) - 1):
            first = jnp.where(u == i, starts[i], first)
            count = jnp.where(u == i, starts[i + 1] - starts[i], count)
        ready = _div(first, per_quarter) * write_rounds

        pl.when(first == 3 * per_quarter)(side_out[1].wait)

        @pl.when(first == batch - 1)
        def _():
            write(sent, before_last)
            side_out[2].wait()
            side_out[3].wait()

        sent = jnp.where(first == batch - 1, before_last, sent)

        def feed_writes(stage, k):
            lo = sent + (stage * count + k) * _STEP_WRITES
            write(lo, jnp.minimum(lo + _STEP_WRITES, ready))

        normalise(first, count, per_quarter, feed_writes)
        return jnp.minimum(sent + 2 * count * _STEP_WRITES, ready)

    lax.fori_loop(0, len(starts) - 1, step, _LEAD_WRITES)

    write(before_last, _QUARTERS * write_rounds)
    for edge, end in zip(edges, edges[1:]):
        edge += write_rounds * _WRITE_BANDS
        if edge < end:
            box = (slice(None), pl.ds(edge, end - edge))
            _copy(buf.at[box], o_hbm.at[box], write_sem).start()
    _copy(buf, o_hbm, write_sem).wait()


@jax.jit
def pallas_standalone__groupnorm__sampling_kernel(
    x: jax.Array,
    g: jax.Array,
    b: jax.Array,
):
    batch, chans, height, width = x.shape
    assert batch == 32 and chans % _GROUPS == 0
    assert pl.cdiv(chans, _LANES) == _STREAMS
    assert batch * height * width == _QUARTERS * _STREAM_TILES * _BAND
    shape = (_QUARTERS, _STREAM_TILES, _BAND, chans)
    in_hbm = pl.BlockSpec(memory_space=pl.ANY)

    out = pl.pallas_call(
        functools.partial(_kernel, batch=batch),
        out_shape=jax.ShapeDtypeStruct(shape, x.dtype),
        in_specs=[in_hbm, in_hbm, in_hbm],
        out_specs=in_hbm,
        scratch_shapes=[
            pltpu.VMEM(shape, x.dtype),
            pltpu.SMEM((_SIDE_SLOTS, _BAND, chans), x.dtype),
            pltpu.VMEM((chans,), g.dtype),
            pltpu.VMEM((chans,), b.dtype),
            pltpu.VMEM((chans,), b.dtype),
            pltpu.VMEM((4, 16, _STREAMS * _LANES), jnp.float32),
            pltpu.SemaphoreType.DMA((4,)),
            pltpu.SemaphoreType.DMA((3,)),
            pltpu.SemaphoreType.DMA((3,)),
            pltpu.SemaphoreType.DMA((4,)),
            pltpu.SemaphoreType.DMA(()),
        ],
        compiler_params=pltpu.CompilerParams(
            vmem_limit_bytes=64 * 1024 * 1024,
            disable_bounds_checks=True,
            disable_semaphore_checks=True,
        ),
    )(jnp.transpose(x, (0, 2, 3, 1)).reshape(shape), g, b)
    return jnp.transpose(out.reshape(batch, height, width, chans), (0, 3, 1, 2))
```
